```python
import jax
import jax.numpy as jnp

def _softmax(x, axis=-1):
    return jax.nn.softmax(x, axis=axis)
def _gelu(x):
    return jax.nn.gelu(x, approximate=True)
def _silu(x):
    return jax.nn.silu(x)
def _sigmoid(x):
    return jax.nn.sigmoid(x)
def _layernorm(x, axis=-1, eps=1e-5):
    m = jnp.mean(x, axis=axis, keepdims=True)
    v = jnp.var(x, axis=axis, keepdims=True)
    return (x - m) / jnp.sqrt(v + eps)
def _scatter_add(tgt, idx, src, axis=0):
    return tgt.at[idx].add(src)
def _segment_sum(src, seg, n):
    return jax.ops.segment_sum(src, seg, n)
class _Rng:
    def __init__(self, key):
        self._k = key
    def _next(self):
        self._k, sub = jax.random.split(self._k)
        return sub
    def normal(self, shape):
        return jax.random.normal(self._next(), shape, dtype=jnp.bfloat16)
    def randint(self, lo, hi, shape):
        return jax.random.randint(self._next(), shape, lo, hi, dtype=jnp.int32)
    def uniform(self, shape, lo=0.0, hi=1.0):
        return jax.random.uniform(self._next(), shape, jnp.bfloat16, lo, hi)
    def permutation(self, n):
        return jax.random.permutation(self._next(), n)


kernel_name = 'gated_mix__compressed_kv_cla__ssm_conv_s5__prompt'

def setup_inputs():
    _rng = _Rng(jax.random.key(int.from_bytes(__import__("os").urandom(4), "little")))
    _w = (lambda a: (lambda t: t.astype(jnp.bfloat16) if jnp.issubdtype(t.dtype, jnp.floating) else t)(jnp.asarray(a)))
    def _A_setup():
        B, H, Sq, Sk, D, M = 1, 16, 2048, 2048, 256, 448
        Dc = 4 * D
        return {
            "x": _w((lambda *s: _rng.normal(s) * 0.05)(B, Sq, M)),
            "c_kv": _w((lambda *s: _rng.normal(s) * 0.05)(B, Sk, Dc)),
            "w_q": _w((lambda *s: _rng.normal(s) * 0.05)(M, H, D) * (M ** -0.5)),
            "w_uk": _w((lambda *s: _rng.normal(s) * 0.05)(Dc, H, D) * (Dc ** -0.5)),
            "w_uv": _w((lambda *s: _rng.normal(s) * 0.05)(Dc, H, D) * (Dc ** -0.5)),
            "w_o": _w((lambda *s: _rng.normal(s) * 0.05)(H, D, M) * ((H * D) ** -0.5)),
        }
    _A_in = _A_setup()

    def _B_setup():
        B, S, D = 1, 2048, 448
        P = D
        Lambda_re = -0.5 * jnp.exp((lambda *s: _rng.normal(s) * 0.05)(P))
        Lambda_im = (lambda *s: _rng.normal(s) * 0.05)(P) * 1.0
        B_re = (lambda *s: _rng.normal(s) * 0.05)(P, D) * (D ** -0.5)
        B_im = (lambda *s: _rng.normal(s) * 0.05)(P, D) * (D ** -0.5)
        C_re = (lambda *s: _rng.normal(s) * 0.05)(D, P) * (P ** -0.5)
        C_im = (lambda *s: _rng.normal(s) * 0.05)(D, P) * (P ** -0.5)
        log_dt = (lambda *s: _rng.normal(s) * 0.05)(P) * 0.3 - 2.0
        Dskip = (lambda *s: _rng.normal(s) * 0.05)(D)
        return {
            "x": _w((lambda *s: _rng.normal(s) * 0.05)(B, S, D)),
            "Lambda_re": _w(Lambda_re),
            "Lambda_im": _w(Lambda_im),
            "B_re": _w(B_re),
            "B_im": _w(B_im),
            "C_re": _w(C_re),
            "C_im": _w(C_im),
            "log_dt": _w(log_dt),
            "Dskip": _w(Dskip),
        }
    _B_in = _B_setup()

    return {
        "A_x": _A_in["x"],
        "A_c_kv": _A_in["c_kv"],
        "A_w_q": _A_in["w_q"],
        "A_w_uk": _A_in["w_uk"],
        "A_w_uv": _A_in["w_uv"],
        "A_w_o": _A_in["w_o"],
        "B_x": _B_in["x"],
        "B_Lambda_re": _B_in["Lambda_re"],
        "B_Lambda_im": _B_in["Lambda_im"],
        "B_B_re": _B_in["B_re"],
        "B_B_im": _B_in["B_im"],
        "B_C_re": _B_in["C_re"],
        "B_C_im": _B_in["C_im"],
        "B_log_dt": _B_in["log_dt"],
        "B_Dskip": _B_in["Dskip"],
        "gate_w": _w((lambda *s: _rng.normal(s) * 0.05)(448)),
    }

def reference(A_x, A_c_kv, A_w_q, A_w_uk, A_w_uv, A_w_o, B_x, B_Lambda_re, B_Lambda_im, B_B_re, B_B_im, B_C_re, B_C_im, B_log_dt, B_Dskip, gate_w):
    def _A_ref(x, c_kv, w_q, w_uk, w_uv, w_o):
        B, Sq, M = x.shape[0], x.shape[1], x.shape[2]
        Sk = c_kv.shape[1]
        H, D = w_q.shape[1], w_q.shape[2]
        q = jnp.einsum("bqm,mhd->bhqd", x, w_q)
        k = jnp.einsum("bkc,chd->bhkd", c_kv, w_uk)
        v = jnp.einsum("bkc,chd->bhkd", c_kv, w_uv)
        scores = jnp.einsum("bhqd,bhkd->bhqk", q, k) * (D ** -0.5)
        off = Sk - Sq
        qi = jnp.arange(Sq)[:, None]
        kj = jnp.arange(Sk)[None, :]
        cmask = kj <= (qi + off)
        scores = jnp.where(cmask[None, None], scores, -1e9)
        p = _softmax(scores, axis=-1)
        ctx = jnp.einsum("bhqk,bhkd->bhqd", p, v)
        return jnp.einsum("bhqd,hdm->bqm", ctx, w_o)

    def _B_ref(x, Lambda_re, Lambda_im, B_re, B_im, C_re, C_im, log_dt, Dskip):
        Bsz, L, H = x.shape
        Lam = Lambda_re + 1j * Lambda_im
        Bmat = B_re + 1j * B_im
        Cmat = C_re + 1j * C_im
        dt = jnp.exp(log_dt)
        Lam_bar = jnp.exp(dt * Lam)
        B_bar = ((Lam_bar - 1.0) / Lam)[:, None] * Bmat
        Bu = jnp.einsum("bld,pd->blp", x + 0j, B_bar)
        h = jnp.zeros_like(Bu[:, 0, :])
        hs = []
        for t in range(L):
            h = Lam_bar[None, :] * h + Bu[:, t, :]
            hs.append(h)
        hseq = jnp.stack(hs, 1)
        y = 2.0 * jnp.einsum("blp,dp->bld", hseq, Cmat).real + x * Dskip[None, None, :]
        return y

    x = A_x
    g = _sigmoid((x * gate_w).sum(-1, keepdims=True))
    a = _A_ref(x, A_c_kv, A_w_q, A_w_uk, A_w_uv, A_w_o)
    b = _B_ref(x, B_Lambda_re, B_Lambda_im, B_B_re, B_B_im, B_C_re, B_C_im, B_log_dt, B_Dskip)
    return g * a + (1 - g) * b
```

```python
import math
import jax
import jax.numpy as jnp
from jax import lax
import jax.experimental.pallas as pl
import jax.experimental.pallas.tpu as pltpu

S, M, H, D, DC, P = 2048, 448, 16, 256, 1024, 448
BQ = 128
NQ = S // BQ
TC = 256
NC = S // TC
F32, BF16, U32 = jnp.float32, jnp.bfloat16, jnp.uint32
NT = (((1,), (1,)), ((), ()))
LOG2E = math.log2(math.e)


def _nt(a, b):
    return lax.dot_general(a, b, NT, preferred_element_type=F32)


def _nn(a, b):
    return jnp.dot(a, b, preferred_element_type=F32)


def _cmul(ar, ai, br, bi):
    return ar * br - ai * bi, ar * bi + ai * br


def _head_w(w32_ref, pair, shift, rows):
    w = jnp.concatenate([w32_ref[u, pl.ds(pair, rows, stride=H // 2), :] for u in range(2)], 1)
    w = (w << shift) & jnp.uint32(0xFFFF0000)
    return pltpu.bitcast(w, F32).astype(BF16)


def _kernel(lre_ref, lim_ref, ldt_ref, dsk_ref, gw_ref,
            xt_hbm, c_hbm, wq_hbm, wk_hbm, wv_hbm, wo_hbm, bre_hbm, bim_hbm, cre_hbm, cim_hbm,
            out_hbm,
            xt_v, c_v, wq_v, wk_v, wv_v, wo_v, bre_v, bim_v, cre_v, cim_v,
            x_s, q_s, k_s, v_s, o_s, wkv_s, g_s, acc_s, coef_s, sems, osem):
    lo = lambda r: r.bitcast(U32).at[:, pl.ds(0, 128)]
    hi = lambda r: r.bitcast(U32).at[:, pl.ds(128, 128)]
    srcs = [xt_hbm, bre_hbm, bim_hbm, lo(wq_hbm), hi(wq_hbm), cre_hbm, cim_hbm,
            c_hbm, lo(wk_hbm), hi(wk_hbm), lo(wv_hbm), hi(wv_hbm), wo_hbm]
    dsts = [xt_v, bre_v, bim_v, wq_v.at[0], wq_v.at[1], cre_v, cim_v,
            c_v, wk_v.at[0], wk_v.at[1], wv_v.at[0], wv_v.at[1], wo_v]
    cps = [pltpu.make_async_copy(s, d, sems.at[i]) for i, (s, d) in enumerate(zip(srcs, dsts))]
    for cp in cps:
        cp.start()

    def row(ref):
        return ref[...].astype(F32).reshape(1, P)

    lre, lim, gw, dsk = row(lre_ref), row(lim_ref), row(gw_ref), row(dsk_ref)
    dt = jnp.exp(row(ldt_ref)).astype(BF16).astype(F32)
    mag = jnp.exp(dt * lre)
    a1r, a1i = mag * jnp.cos(dt * lim), mag * jnp.sin(dt * lim)
    den = lre * lre + lim * lim
    cr = ((a1r - 1.0) * lre + a1i * lim) / den
    ci = (a1i * lre - (a1r - 1.0) * lim) / den
    a2r, a2i = _cmul(a1r, a1i, a1r, a1i)
    a4r, a4i = _cmul(a2r, a2i, a2r, a2i)
    r8 = lax.broadcasted_iota(jnp.int32, (8, P), 0)
    bc = lambda v: jnp.broadcast_to(v, (8, P))
    for n, (k, vr, vi) in enumerate(((1, a1r, a1i), (2, a2r, a2i), (4, a4r, a4i))):
        coef_s[2 * n] = jnp.where(r8 >= k, bc(vr), 0.0)
        coef_s[2 * n + 1] = jnp.where(r8 >= k, bc(vi), 0.0)
    pr, pi = bc(a1r), bc(a1i)
    for k, vr, vi in ((1, a1r, a1i), (2, a2r, a2i), (4, a4r, a4i)):
        nr, ni = _cmul(pr, pi, bc(vr), bc(vi))
        pr, pi = jnp.where((r8 & k) != 0, nr, pr), jnp.where((r8 & k) != 0, ni, pi)
    coef_s[6], coef_s[7] = pr, pi
    coef_s[8], coef_s[9] = bc(cr), bc(ci)
    col = lambda v: jnp.broadcast_to(v, (128, P)).T
    gw_col, dsk_col = col(gw), col(dsk)

    cps[0].wait()
    x_s[...] = xt_v[...].T
    for cp in cps[1:7]:
        cp.wait()
    wq32 = wq_v
    wk32 = wk_v
    wv32 = wv_v

    def gate(z):
        z = z.astype(BF16).astype(F32)
        return (1.0 / (1.0 + jnp.exp(-z))).astype(BF16).astype(F32)

    def phase1(i, carry):
        for par in range(2):
            w = _head_w(wq32, i, jnp.uint32(16 - 16 * par), M)
            q_s[2 * i + par] = (_nn(x_s[...], w) * (D ** -0.5 * LOG2E)).astype(BF16)
        t0 = pl.multiple_of(i * TC, TC)
        xc = x_s[pl.ds(t0, TC), :]
        zc = jnp.sum((xc.astype(F32) * gw).astype(BF16).astype(F32), axis=1, keepdims=True)
        g_s[pl.ds(t0, TC), :] = jnp.broadcast_to(gate(zc), (TC, 128))
        ur, ui = _nt(xc, bre_v[...]), _nt(xc, bim_v[...])
        hr_c, hi_c = carry
        cf = [coef_s[n] for n in range(10)]
        hrs, his = [], []
        for j in range(TC // 8):
            br, bi = _cmul(ur[8 * j:8 * j + 8], ui[8 * j:8 * j + 8], cf[8], cf[9])
            for n, k in enumerate((1, 2, 4)):
                sr, si = _cmul(pltpu.roll(br, k, 0), pltpu.roll(bi, k, 0), cf[2 * n], cf[2 * n + 1])
                br, bi = br + sr, bi + si
            sr, si = _cmul(hr_c, hi_c, cf[6], cf[7])
            br, bi = br + sr, bi + si
            hr_c, hi_c = bc(br[7:8]), bc(bi[7:8])
            hrs.append(br)
            his.append(bi)
        hr = jnp.concatenate(hrs, 0).astype(BF16)
        hi = jnp.concatenate(his, 0).astype(BF16)
        yt = 2.0 * (_nt(cre_v[...], hr) - _nt(cim_v[...], hi))
        for u in range(TC // 128):
            xtc = xt_v[:, pl.ds(pl.multiple_of(t0 + 128 * u, 128), 128)].astype(F32)
            zr = jnp.sum((xtc * gw_col).astype(BF16).astype(F32), axis=0, keepdims=True)
            omg = (1.0 - gate(zr)).astype(BF16).astype(F32)
            acc_s[i * (TC // 128) + u] = omg * (yt[:, 128 * u:128 * u + 128] + xtc * dsk_col)
        return hr_c, hi_c

    z8 = jnp.zeros((8, P), F32)
    lax.fori_loop(0, NC, phase1, (z8, z8))
    for cp in cps[7:]:
        cp.wait()

    tri = (lax.broadcasted_iota(jnp.int32, (BQ, BQ), 1) <= lax.broadcasted_iota(jnp.int32, (BQ, BQ), 0))

    def head(h, _):
        pair = h // 2
        shift = (16 - 16 * (h % 2)).astype(U32)
        wkv_s[:, :D] = _head_w(wk32, pair, shift, DC)
        wkv_s[:, D:] = _head_w(wv32, pair, shift, DC)
        kv = _nn(c_v[...], wkv_s[...]).astype(BF16)
        k_s[...] = kv[:, :D]
        v_s[...] = kv[:, D:]

        def st_a(i):
            q = q_s[h, BQ * i:BQ * (i + 1), :]
            s = _nt(q, k_s[:BQ * (i + 1), :])
            sd = jnp.where(tri, s[:, BQ * i:], -1e9 * LOG2E)
            s = jnp.concatenate([s[:, :BQ * i], sd], 1) if i else sd
            return s, jnp.max(s, axis=1, keepdims=True)

        def st_b(i, s, m):
            p = jnp.exp2(s - m)
            l = jnp.sum(p, axis=1, keepdims=True)
            o = _nn(p.astype(BF16), v_s[:BQ * (i + 1), :])
            w = g_s[BQ * i:BQ * (i + 1), :] / l
            o = (o * jnp.concatenate([w, w], 1)).astype(BF16)
            acc_s[i] += _nt(wo_v[h], o)

        for i in range(NQ):
            st_b(i, *st_a(i))
        return 0

    lax.fori_loop(0, H, head, 0)
    ocs = [pltpu.make_async_copy(acc_s.at[i], out_hbm.at[:, pl.ds(BQ * i, BQ)], osem.at[i]) for i in range(NQ)]
    for cp in ocs:
        cp.start()
    for cp in ocs:
        cp.wait()


@jax.jit
def pallas_gated_mix__compressed_kv_cla__ssm_conv_s5__prompt_kernel(A_x, A_c_kv, A_w_q, A_w_uk, A_w_uv, A_w_o, B_x, B_Lambda_re, B_Lambda_im, B_B_re, B_B_im,
              B_C_re, B_C_im, B_log_dt, B_Dskip, gate_w):
    vm = pl.BlockSpec(memory_space=pltpu.VMEM)
    hbm = pl.BlockSpec(memory_space=pl.ANY)
    big = [A_x[0].T, A_c_kv[0], A_w_q.reshape(M * H, D), A_w_uk.reshape(DC * H, D), A_w_uv.reshape(DC * H, D),
           jnp.swapaxes(A_w_o, 1, 2), B_B_re, B_B_im, B_C_re, B_C_im]
    V = pltpu.VMEM
    out_t = pl.pallas_call(
        _kernel,
        in_specs=[vm] * 5 + [hbm] * 10,
        out_specs=hbm,
        out_shape=jax.ShapeDtypeStruct((M, S), F32),
        scratch_shapes=[V((2, a.shape[0] // 2, 128), U32) if a.shape[-1] == D and a.ndim == 2 else V(a.shape, BF16) for a in big] + [
            V((S, M), BF16), V((H, S, D), BF16), V((S, D), BF16), V((S, D), BF16), V((S, D), BF16),
            V((DC, 2 * D), BF16), V((S, 128), F32), V((NQ, M, BQ), F32), V((10, 8, P), F32),
            pltpu.SemaphoreType.DMA((13,)), pltpu.SemaphoreType.DMA((NQ,))],
        compiler_params=pltpu.CompilerParams(vmem_limit_bytes=110 << 20),
    )(B_Lambda_re, B_Lambda_im, B_log_dt, B_Dskip, gate_w, *big)
    return out_t.T[None]
```

```python
import math
import jax
import jax.numpy as jnp
from jax import lax
import jax.experimental.pallas as pl
import jax.experimental.pallas.tpu as pltpu

S, M, H, D, DC, P = 2048, 448, 16, 256, 1024, 448
BQ = 128
NQ = S // BQ
TC = 256
NC = S // TC
OC = TC
LAG, KVS = 3, 1
F32, BF16, U32 = jnp.float32, jnp.bfloat16, jnp.uint32
NT = (((1,), (1,)), ((), ()))
LOG2E = math.log2(math.e)


def _nt(a, b):
    return lax.dot_general(a, b, NT, preferred_element_type=F32)


def _nn(a, b):
    return jnp.dot(a, b, preferred_element_type=F32)


def _cmul(ar, ai, br, bi):
    return ar * br - ai * bi, ar * bi + ai * br


def _head_w(w32_ref, pair, shift, rows):
    w = jnp.concatenate([w32_ref[u, pl.ds(pair, rows, stride=H // 2), :] for u in range(2)], 1)
    w = (w << shift) & jnp.uint32(0xFFFF0000)
    return pltpu.bitcast(w, F32).astype(BF16)


def _kernel(lre_ref, lim_ref, ldt_ref, dsk_ref, gw_ref,
            xt_hbm, c_hbm, wq_hbm, wk_hbm, wv_hbm, wo_hbm, bre_hbm, bim_hbm, cre_hbm, cim_hbm,
            out_hbm,
            xt_v, c_v, wq_v, wk_v, wv_v, wo_v, bre_v, bim_v, cre_v, cim_v,
            x_s, q_s, k_s, v_s, bu_s, wkv_s, g_s, acc_s, coef_s, h_s, sems, osem):
    lo = lambda r: r.bitcast(U32).at[:, pl.ds(0, 128)]
    hi = lambda r: r.bitcast(U32).at[:, pl.ds(128, 128)]
    srcs = [xt_hbm, bre_hbm, bim_hbm, lo(wq_hbm), hi(wq_hbm), cre_hbm, cim_hbm,
            c_hbm, lo(wk_hbm), hi(wk_hbm), lo(wv_hbm), hi(wv_hbm), wo_hbm]
    dsts = [xt_v, bre_v, bim_v, wq_v.at[0], wq_v.at[1], cre_v, cim_v,
            c_v, wk_v.at[0], wk_v.at[1], wv_v.at[0], wv_v.at[1], wo_v]
    cps = [pltpu.make_async_copy(s, d, sems.at[i]) for i, (s, d) in enumerate(zip(srcs, dsts))]
    for cp in cps[:3]:
        cp.start()

    def row(ref):
        return ref[...].astype(F32).reshape(1, P)

    lre, lim, gw, dsk = row(lre_ref), row(lim_ref), row(gw_ref), row(dsk_ref)
    dt = jnp.exp(row(ldt_ref)).astype(BF16).astype(F32)
    mag = jnp.exp(dt * lre)
    a1r, a1i = mag * jnp.cos(dt * lim), mag * jnp.sin(dt * lim)
    den = lre * lre + lim * lim
    cr = ((a1r - 1.0) * lre + a1i * lim) / den
    ci = (a1i * lre - (a1r - 1.0) * lim) / den
    a2r, a2i = _cmul(a1r, a1i, a1r, a1i)
    a4r, a4i = _cmul(a2r, a2i, a2r, a2i)
    r8 = lax.broadcasted_iota(jnp.int32, (8, P), 0)
    bc = lambda v: jnp.broadcast_to(v, (8, P))
    for n, (k, vr, vi) in enumerate(((1, a1r, a1i), (2, a2r, a2i), (4, a4r, a4i))):
        coef_s[2 * n] = jnp.where(r8 >= k, bc(vr), 0.0)
        coef_s[2 * n + 1] = jnp.where(r8 >= k, bc(vi), 0.0)
    pr, pi = bc(a1r), bc(a1i)
    for k, vr, vi in ((1, a1r, a1i), (2, a2r, a2i), (4, a4r, a4i)):
        nr, ni = _cmul(pr, pi, bc(vr), bc(vi))
        pr, pi = jnp.where((r8 & k) != 0, nr, pr), jnp.where((r8 & k) != 0, ni, pi)
    coef_s[6], coef_s[7] = pr, pi
    col = lambda v: jnp.broadcast_to(v, (128, P)).T
    gw_col, dsk_col = col(gw), col(dsk)

    for cp in cps[:3]:
        cp.wait()
    for cp in cps[3:7]:
        cp.start()

    def gate(z):
        z = z.astype(BF16).astype(F32)
        return (1.0 / (1.0 + jnp.exp(-z))).astype(BF16).astype(F32)

    @pl.loop(0, 2)
    def _(o):
      for i in range(NC // 2):
        r = pl.ds(pl.multiple_of(o * (S // 2) + TC * i, TC), TC)
        xc = xt_v[:, r].T
        x_s[r, :] = xc
        zc = jnp.sum((xc.astype(F32) * gw).astype(BF16).astype(F32), axis=1, keepdims=True)
        g_s[r, :] = jnp.broadcast_to(gate(zc), (TC, 128))
        bu_s[0, r, :] = _nt(xc, bre_v[...])
        bu_s[1, r, :] = _nt(xc, bim_v[...])
    for cp in cps[3:7]:
        cp.wait()
    for cp in cps[7:]:
        cp.start()
    c2r, c2i = jnp.broadcast_to(2.0 * cr, (16, P)), jnp.broadcast_to(2.0 * ci, (16, P))

    @pl.loop(0, M // 64)
    def _(n):
        for e in range(4):
            r = pl.ds(pl.multiple_of(64 * n + 16 * e, 16), 16)
            er, ei = _cmul(cre_v[r, :].astype(F32), cim_v[r, :].astype(F32), c2r, c2i)
            cre_v[r, :] = er.astype(BF16)
            cim_v[r, :] = (-ei).astype(BF16)
    wq32 = wq_v
    wk32 = wk_v
    wv32 = wv_v

    def phase1(i, carry):
        w = jnp.concatenate([_head_w(wq32, i, jnp.uint32(16 - 16 * par), M) for par in range(2)], 1)

        def qproj(n):
            r = slice(128 * n, 128 * (n + 1))
            q = (_nn(x_s[r, :], w) * (D ** -0.5 * LOG2E)).astype(BF16)
            q_s[2 * i, r, :] = q[:, :D]
            q_s[2 * i + 1, r, :] = q[:, D:]

        qproj(0)
        t0 = pl.multiple_of(i * TC, TC)
        hr_c, hi_c = carry
        for j in range(TC // 16):
            r = pl.ds(pl.multiple_of(t0 + 16 * j, 16), 16)
            ur, ui = bu_s[0, r, :], bu_s[1, r, :]
            cf = [coef_s[n] for n in range(8)]
            hrs, his = [], []
            for e in range(2):
                br, bi = ur[8 * e:8 * e + 8], ui[8 * e:8 * e + 8]
                for n, k in enumerate((1, 2, 4)):
                    sr, si = _cmul(pltpu.roll(br, k, 0), pltpu.roll(bi, k, 0), cf[2 * n], cf[2 * n + 1])
                    br, bi = br + sr, bi + si
                sr, si = _cmul(hr_c, hi_c, cf[6], cf[7])
                br, bi = br + sr, bi + si
                hr_c, hi_c = bc(br[7:8]), bc(bi[7:8])
                hrs.append(br)
                his.append(bi)
            omg = (1.0 - g_s[r, :]).astype(BF16).astype(F32)
            omg = jnp.concatenate([omg] * 4, 1)[:, :P]
            h_s[0, r, :] = (jnp.concatenate(hrs, 0) * omg).astype(BF16)
            h_s[1, r, :] = (jnp.concatenate(his, 0) * omg).astype(BF16)
            if j + 1 < 16:
                qproj(j + 1)
        for u in range(TC // 128):
            xtc = xt_v[:, pl.ds(pl.multiple_of(t0 + 128 * u, 128), 128)].astype(F32)
            zr = jnp.sum((xtc * gw_col).astype(BF16).astype(F32), axis=0, keepdims=True)
            omg = (1.0 - gate(zr)).astype(BF16).astype(F32)
            acc_s[i, :, 128 * u:128 * u + 128] = omg * (xtc * dsk_col)
        return hr_c, hi_c

    z8 = jnp.zeros((8, P), F32)
    lax.fori_loop(0, NC, phase1, (z8, z8))
    for cp in cps[7:]:
        cp.wait()
    tri = (lax.broadcasted_iota(jnp.int32, (BQ, BQ), 1) <= lax.broadcasted_iota(jnp.int32, (BQ, BQ), 0))

    def prep(h):
        pair = h // 2
        shift = jnp.asarray(16 - 16 * (h % 2)).astype(U32)
        wkv_s[:, :D] = _head_w(wk32, pair, shift, DC)
        wkv_s[:, D:] = _head_w(wv32, pair, shift, DC)

    def st_kv(lo, hi):
        kv = _nn(c_v[lo:hi, :], wkv_s[...]).astype(BF16)
        k_s[lo:hi, :] = kv[:, :D]
        v_s[lo:hi, :] = kv[:, D:]

    def head(h):
        prep(h)

        def st_a(i):
            q = q_s[h, BQ * i:BQ * (i + 1), :]
            s = _nt(q, k_s[:BQ * (i + 1), :])
            sd = jnp.where(tri, s[:, BQ * i:], -1e9 * LOG2E)
            s = jnp.concatenate([s[:, :BQ * i], sd], 1) if i else sd
            return s, jnp.max(s, axis=1, keepdims=True)

        def st_b(i, s, m):
            p = jnp.exp2(s - m)
            l = jnp.sum(p, axis=1, keepdims=True)
            return p.astype(BF16), g_s[BQ * i:BQ * (i + 1), :] / l

        def st_c(i, p, w):
            o = _nn(p, v_s[:BQ * (i + 1), :])
            q_s[h, BQ * i:BQ * (i + 1), :] = (o * jnp.concatenate([w, w], 1)).astype(BF16)

        st_kv(0, 2 * BQ)
        done = 2
        ra, rb = {}, {}
        nc = 0
        for t in range(NQ + LAG):
            if 0 <= t - 1 < NQ: rb[t - 1] = st_b(t - 1, *ra.pop(t - 1))
            lag = 2 if done < NQ else LAG
            if nc <= t - lag:
                st_c(nc, *rb.pop(nc))
                nc += 1
            if t < NQ: ra[t] = st_a(t)
            if done < NQ:
                st_kv(done * BQ, (done + KVS) * BQ)
                done += KVS
        assert nc == NQ
        return 0

    lax.fori_loop(0, H, lambda h, _: head(h), 0)

    def ocp(i):
        return pltpu.make_async_copy(acc_s.at[i], out_hbm.at[:, pl.ds(pl.multiple_of(i * OC, OC), OC)], osem.at[i])

    def final(i, _):
        r = pl.ds(pl.multiple_of(i * OC, OC), OC)
        acc = acc_s[i] + _nt(cre_v[...], h_s[0, r, :]) + _nt(cim_v[...], h_s[1, r, :])
        for h in range(H):
            acc += _nt(wo_v[h], q_s[h, r, :])
        acc_s[i] = acc
        ocp(i).start()
        return 0

    lax.fori_loop(0, S // OC, final, 0)
    for i in range(S // OC):
        ocp(i).wait()


@jax.jit
def pallas_gated_mix__compressed_kv_cla__ssm_conv_s5__prompt_kernel(A_x, A_c_kv, A_w_q, A_w_uk, A_w_uv, A_w_o, B_x, B_Lambda_re, B_Lambda_im, B_B_re, B_B_im,
              B_C_re, B_C_im, B_log_dt, B_Dskip, gate_w):
    vm = pl.BlockSpec(memory_space=pltpu.VMEM)
    hbm = pl.BlockSpec(memory_space=pl.ANY)
    big = [A_x[0].T, A_c_kv[0], A_w_q.reshape(M * H, D), A_w_uk.reshape(DC * H, D), A_w_uv.reshape(DC * H, D),
           jnp.swapaxes(A_w_o, 1, 2), B_B_re, B_B_im, B_C_re, B_C_im]
    V = pltpu.VMEM
    out_t = pl.pallas_call(
        _kernel,
        in_specs=[vm] * 5 + [hbm] * 10,
        out_specs=hbm,
        out_shape=jax.ShapeDtypeStruct((M, S), F32),
        scratch_shapes=[V((2, a.shape[0] // 2, 128), U32) if a.shape[-1] == D and a.ndim == 2 else V(a.shape, BF16) for a in big] + [
            V((S, M), BF16), V((H, S, D), BF16), V((S, D), BF16), V((S, D), BF16), V((2, S, P), F32),
            V((DC, 2 * D), BF16), V((S, 128), F32), V((NC, M, TC), F32), V((8, 8, P), F32), V((2, S, P), BF16),
            pltpu.SemaphoreType.DMA((13,)), pltpu.SemaphoreType.DMA((NQ,))],
        compiler_params=pltpu.CompilerParams(vmem_limit_bytes=110 << 20),
    )(B_Lambda_re, B_Lambda_im, B_log_dt, B_Dskip, gate_w, *big)
    return out_t.T[None]
```
